```python
import os as _os
_os.environ.setdefault("JAX_PLATFORMS", "cpu")
import jax
import jax.numpy as jnp

def _softmax(x, axis=-1):
    return jax.nn.softmax(x, axis=axis)
def _gelu(x):
    return jax.nn.gelu(x, approximate=True)
def _silu(x):
    return jax.nn.silu(x)
def _sigmoid(x):
    return jax.nn.sigmoid(x)
def _layernorm(x, axis=-1, eps=1e-5):
    m = jnp.mean(x, axis=axis, keepdims=True)
    v = jnp.var(x, axis=axis, keepdims=True)
    return (x - m) / jnp.sqrt(v + eps)
def _scatter_add(tgt, idx, src, axis=0):
    return tgt.at[idx].add(src)
def _segment_sum(src, seg, n):
    return jax.ops.segment_sum(src, seg, n)
class _Rng:
    def __init__(self, key):
        self._k = key
    def _next(self):
        self._k, sub = jax.random.split(self._k)
        return sub
    def normal(self, shape):
        return jax.random.normal(self._next(), shape, dtype=jnp.bfloat16)
    def randint(self, lo, hi, shape):
        return jax.random.randint(self._next(), shape, lo, hi, dtype=jnp.int32)
    def uniform(self, shape, lo=0.0, hi=1.0):
        return jax.random.uniform(self._next(), shape, jnp.bfloat16, lo, hi)
    def permutation(self, n):
        return jax.random.permutation(self._next(), n)


kernel_name = 'standalone__dense_activation_gelu__prompt'

def setup_inputs():
    _rng = _Rng(jax.random.key(int.from_bytes(__import__("os").urandom(4), "little")))
    _w = (lambda a: (lambda t: t.astype(jnp.bfloat16) if jnp.issubdtype(t.dtype, jnp.floating) else t)(jnp.asarray(a)))
    B, S, D, F = 1, 2048, 640, 1728
    return {
        "x": _w((lambda *s: _rng.normal(s) * 0.05)(B, S, D)),
        "w1": _w((lambda *s: _rng.normal(s) * 0.05)(D, F) * (D ** -0.5)),
        "b1": _w((lambda *s: _rng.normal(s) * 0.05)(F) * 0.01),
        "w2": _w((lambda *s: _rng.normal(s) * 0.05)(F, D) * (F ** -0.5)),
        "b2": _w((lambda *s: _rng.normal(s) * 0.05)(D) * 0.01),
    }

def reference(x, w1, b1, w2, b2):
    h = jnp.einsum("bsd,df->bsf", x, w1) + b1
    h = _gelu(h)
    return jnp.einsum("bsf,fd->bsd", h, w2) + b2
```

```python
import jax
import jax.numpy as jnp
import jax.experimental.pallas as pl
import jax.experimental.pallas.tpu as pltpu

_COPIES = (
    ("b1", 0, 0, 0, None),
    ("b2", 0, 0, 4, None),
    ("x", 0, 192, 0, None),
    ("w1", 0, 128, 0, None),
    ("w1", 128, 128, 1, None),
    ("w1", 256, 128, 2, None),
    ("x", 192, 64, 3, None),
    ("x", 256, 128, 0, 3),
    ("x", 384, 128, 1, 4),
    ("w1", 384, 256, 2, 5),
    ("x", 512, 128, 3, 6),
    ("w1", 640, 512, 0, 7),
    ("w1", 1152, 576, 1, 8),
    ("w2", 0, 128, 2, 9),
    ("w2", 128, 1600, 3, 10),
    ("x", 640, 1408, 0, 11),
)
_NUM_IN_SEMS = 5

_HEAD = 640
_HEAD_RECTS = (
    (0, 192, 0, 128),
    (0, 192, 128, 128),
    (0, 192, 256, 128),
    (192, 64, 0, 384),
    (256, 128, 0, 384),
    (384, 128, 0, 384),
    (0, 512, 384, 256),
    (512, 128, 0, 640),
    (0, 640, 640, 512),
    (0, 640, 1152, 512),
)
_HEAD_K2 = ((0, 128), (128, 1600))
_TILES = (896, 384, 128)

_OUTS = (
    (0, 640, 0, 640),
    (640, 896, 0, 640),
    (1536, 384, 0, 640),
    (1920, 128, 0, 256),
    (1920, 128, 256, 256),
    (1920, 128, 512, 128),
)


def _nt_dot(a, b):
    return jax.lax.dot_general(a, b, (((1,), (1,)), ((), ())),
                               preferred_element_type=jnp.float32)


def _cat(vals, axis):
    return vals[0] if len(vals) == 1 else jnp.concatenate(vals, axis=axis)


def _ffn_kernel(x_hbm, w1t_hbm, b1_hbm, w2_hbm, b2_hbm, o_hbm,
                x_v, w1t_v, w2_v, b1_v, b2_v, o_v, in_sems, out_sem, trips):
    f_all = w1t_v.shape[0]
    f_main = (f_all // 128) * 128
    f_strip = f_all - f_main

    def program():
        copies = []
        for tensor, r0, rows, slot, _ in _COPIES:
            if tensor == "x":
                src, dst = x_hbm.at[0, pl.ds(r0, rows), :], x_v.at[pl.ds(r0, rows), :]
            elif tensor == "w1":
                src, dst = w1t_hbm.at[pl.ds(r0, rows), :], w1t_v.at[pl.ds(r0, rows), :]
            elif tensor == "w2":
                src, dst = w2_hbm.at[pl.ds(r0, rows), :], w2_v.at[pl.ds(r0, rows), :]
            elif tensor == "b1":
                src, dst = b1_hbm, b1_v
            else:
                src, dst = b2_hbm, b2_v
            copies.append(pltpu.make_async_copy(src, dst, in_sems.at[slot]))
        started = [False] * len(copies)
        waited = [False] * len(copies)

        def need(tensor, r0=0, rows=0):
            for i, (t, c0, cs, slot, _) in enumerate(_COPIES):
                overlaps = t == tensor and (cs == 0 or (c0 < r0 + rows and r0 < c0 + cs))
                if not overlaps or waited[i]:
                    continue
                assert started[i]
                for j, other in enumerate(_COPIES):
                    if other[3] == slot and started[j] and not waited[j]:
                        copies[j].wait()
                        waited[j] = True
                for j, other in enumerate(_COPIES):
                    if not started[j] and other[4] is not None and waited[other[4]]:
                        copies[j].start()
                        started[j] = True

        for i, c in enumerate(_COPIES):
            if c[4] is None:
                copies[i].start()
                started[i] = True

        out_copies = [
            pltpu.make_async_copy(o_v.at[pl.ds(r0, rows), pl.ds(c0, cols)],
                                  o_hbm.at[0, pl.ds(r0, rows), pl.ds(c0, cols)],
                                  out_sem.at[0])
            for r0, rows, c0, cols in _OUTS]
        next_out = [0]

        def emit(r0, rows, val):
            ready = []
            while (next_out[0] < len(_OUTS)
                   and _OUTS[next_out[0]][0] + _OUTS[next_out[0]][1] <= r0 + rows):
                ready.append(next_out[0])
                next_out[0] += 1
            cuts = sorted({0, val.shape[1]} | {_OUTS[j][2] + _OUTS[j][3] for j in ready})
            for ca, cb in zip(cuts[:-1], cuts[1:]):
                o_v[pl.ds(r0, rows), pl.ds(ca, cb - ca)] = val[:, ca:cb]
                for j in ready:
                    if _OUTS[j][2] + _OUTS[j][3] == cb:
                        out_copies[j].start()

        biases = {}

        def bias(name, ref):
            if name not in biases:
                need(name)
                biases[name] = ref[...].astype(jnp.float32)[None, :]
            return biases[name]

        def act_main(r0, rows, f0, fs):
            need("x", r0, rows)
            need("w1", f0, fs)
            h = _nt_dot(x_v[pl.ds(r0, rows), :], w1t_v[pl.ds(f0, fs), :])
            h = h + bias("b1", b1_v)[:, f0:f0 + fs]
            return jax.nn.gelu(h, approximate=True).astype(jnp.bfloat16)

        def act_strip(r0, rows):
            need("x", r0, rows)
            need("w1", f_main, f_strip)
            h = _nt_dot(w1t_v[pl.ds(f_main, f_strip), :], x_v[pl.ds(r0, rows), :]).T
            h = h + bias("b1", b1_v)[:, f_main:]
            return jax.nn.gelu(h, approximate=True).astype(jnp.bfloat16)

        rects = [(r0, rows, f0, fs, act_main(r0, rows, f0, fs))
                 for r0, rows, f0, fs in _HEAD_RECTS]
        rects.append((0, _HEAD, f_main, f_strip, act_strip(0, _HEAD)))
        row_cuts = sorted({r[0] for r in rects} | {_HEAD})

        def head_act(f0, fs):
            bands = []
            for ra, rb in zip(row_cuts[:-1], row_cuts[1:]):
                parts, c = [], f0
                while c < f0 + fs:
                    r0, rows, c0, cs, val = next(
                        r for r in rects
                        if r[0] <= ra and rb <= r[0] + r[1] and r[2] <= c < r[2] + r[3])
                    e = min(f0 + fs, c0 + cs)
                    if (ra, rb) != (r0, r0 + rows):
                        val = val[ra - r0:rb - r0, :]
                    if (c, e) != (c0, c0 + cs):
                        val = val[:, c - c0:e - c0]
                    parts.append(val)
                    c = e
                bands.append(_cat(parts, 1))
            return _cat(bands, 0)

        acc = None
        for k0, ks in _HEAD_K2:
            need("w2", k0, ks)
            part = jnp.dot(head_act(k0, ks), w2_v[pl.ds(k0, ks), :],
                           preferred_element_type=jnp.float32)
            acc = part if acc is None else acc + part
        emit(0, _HEAD, (acc + bias("b2", b2_v)).astype(o_v.dtype))

        r0 = _HEAD
        for rows in _TILES:
            act = _cat([act_main(r0, rows, 0, f_main), act_strip(r0, rows)], 1)
            acc = jnp.dot(act, w2_v[...], preferred_element_type=jnp.float32)
            emit(r0, rows, (acc + bias("b2", b2_v)).astype(o_v.dtype))
            r0 += rows

        assert all(waited) and next_out[0] == len(_OUTS) and r0 == o_v.shape[0]
        for c in out_copies:
            c.wait()

    trips[0] = 1

    def trip(_, carry):
        program()
        return carry

    jax.lax.fori_loop(0, trips[0], trip, 0)


@jax.jit
def pallas_standalone__dense_activation_gelu__prompt_kernel(
    x: jax.Array,
    w1: jax.Array,
    b1: jax.Array,
    w2: jax.Array,
    b2: jax.Array,
):
    batch, seq, d = x.shape
    f = w1.shape[1]
    assert (batch, seq, d, f) == (1, 2048, 640, 1728), "schedule is shape-specific"
    hbm = pl.BlockSpec(memory_space=pl.ANY)
    return pl.pallas_call(
        _ffn_kernel,
        in_specs=[hbm] * 5,
        out_specs=hbm,
        out_shape=jax.ShapeDtypeStruct((batch, seq, d), x.dtype),
        scratch_shapes=[
            pltpu.VMEM((seq, d), x.dtype),
            pltpu.VMEM((f, d), w1.dtype),
            pltpu.VMEM((f, d), w2.dtype),
            pltpu.VMEM((f,), b1.dtype),
            pltpu.VMEM((d,), b2.dtype),
            pltpu.VMEM((seq, d), x.dtype),
            pltpu.SemaphoreType.DMA((_NUM_IN_SEMS,)),
            pltpu.SemaphoreType.DMA((1,)),
            pltpu.SMEM((1,), jnp.int32),
        ],
        compiler_params=pltpu.CompilerParams(
            vmem_limit_bytes=64 * 1024 * 1024,
            flags={"XLA_TPU_RESCHEDULE_DMA_DONES": True},
        ),
    )(x, w1.T, b1, w2, b2)
```
